```python
import os as _os
_os.environ.setdefault("JAX_PLATFORMS", "cpu")
import jax
import jax.numpy as jnp

def _softmax(x, axis=-1):
    return jax.nn.softmax(x, axis=axis)
def _gelu(x):
    return jax.nn.gelu(x, approximate=True)
def _silu(x):
    return jax.nn.silu(x)
def _sigmoid(x):
    return jax.nn.sigmoid(x)
def _layernorm(x, axis=-1, eps=1e-5):
    m = jnp.mean(x, axis=axis, keepdims=True)
    v = jnp.var(x, axis=axis, keepdims=True)
    return (x - m) / jnp.sqrt(v + eps)
def _scatter_add(tgt, idx, src, axis=0):
    return tgt.at[idx].add(src)
def _segment_sum(src, seg, n):
    return jax.ops.segment_sum(src, seg, n)
class _Rng:
    def __init__(self, key):
        self._k = key
    def _next(self):
        self._k, sub = jax.random.split(self._k)
        return sub
    def normal(self, shape):
        return jax.random.normal(self._next(), shape, dtype=jnp.bfloat16)
    def randint(self, lo, hi, shape):
        return jax.random.randint(self._next(), shape, lo, hi, dtype=jnp.int32)
    def uniform(self, shape, lo=0.0, hi=1.0):
        return jax.random.uniform(self._next(), shape, jnp.bfloat16, lo, hi)
    def permutation(self, n):
        return jax.random.permutation(self._next(), n)


kernel_name = 'standalone__dcn_v2_cross__recsys'

def setup_inputs():
    _rng = _Rng(jax.random.key(int.from_bytes(__import__("os").urandom(4), "little")))
    _w = (lambda a: (lambda t: t.astype(jnp.bfloat16) if jnp.issubdtype(t.dtype, jnp.floating) else t)(jnp.asarray(a)))
    B, F, D, L = 4096, 26, 128, 6
    Din = min(F * D, 1024)
    return {
        "x0": _w((lambda *s: _rng.normal(s) * 0.05)(B, Din)),
        "ws": _w((lambda *s: _rng.normal(s) * 0.05)(L, Din, Din)),
        "bs": _w((lambda *s: _rng.normal(s) * 0.05)(L, Din)),
    }

def reference(x0, ws, bs):
    x = x0
    for l in range(ws.shape[0]):
        x = x0 * (x @ ws[l] + bs[l]) + x
    return x
```

```python
import jax, jax.numpy as jnp
import jax.experimental.pallas as pl
import jax.experimental.pallas.tpu as pltpu
f32, bf16 = jnp.float32, jnp.bfloat16

AC = [((0,1),), ((3,1),), ((0,1),(3,1)), ((1,1),(3,-1)), ((2,1),(0,-1)), ((0,1),(1,1)), ((2,1),(3,1))]
BC = [((1,1),(3,-1)), ((2,1),(0,-1)), ((0,1),(3,1)), ((2,1),(3,1)), ((0,1),(1,1)), ((3,1),), ((0,1),)]
CC = [((1,1),(3,1)), ((0,1),(2,1)), ((0,1),(3,1)), ((0,1),), ((3,1),), ((0,-1),(1,1)), ((2,1),(3,-1))]

ORD = [0, 5, 1, 6, 2, 3, 4]
AC, BC, CC = ([t[i] for i in ORD] for t in (AC, BC, CC))
class Neg:
    def __init__(s, v): s.v = v
    def __add__(s, o): return o - s.v
def comb(c, q):
    (i, s) = c[0]
    assert s == 1
    if len(c) == 1: return q[i]
    (j, t) = c[1]
    return q[i] + q[j] if t == 1 else q[i] - q[j]

def quads(blk):
    h = len(blk) // 2
    return [[r[:h] for r in blk[:h]], [r[h:] for r in blk[:h]], [r[:h] for r in blk[h:]], [r[h:] for r in blk[h:]]]
def emap(f, *bs):
    return [[f(*e) for e in zip(*rs)] for rs in zip(*bs)]

def combos(blk, T):
    if len(blk) == 1:
        yield blk[0][0]; return
    q = quads(blk)
    for c in T:
        sub = emap(lambda *e: comb(c, e), *q)
        yield from combos(sub, T)

def products(n, it):
    if n == 1: return [[next(it)]]
    C = [None] * 4
    for c in CC:
        m = products(n // 2, it)
        for (i, s) in c:
            if C[i] is None: C[i] = m if s == 1 else emap(Neg, m)
            else: C[i] = emap((lambda a, b: a + b) if s == 1 else (lambda a, b: a - b), C[i], m)
    return [a + b for a, b in zip(C[0], C[1])] + [a + b for a, b in zip(C[2], C[3])]

@jax.jit
def pallas_standalone__dcn_v2_cross__recsys_kernel(x0, ws, bs):
    bm, lev = 512, 2
    B, D = x0.shape
    L = ws.shape[0]
    n = 2 ** lev; P = 7 ** lev
    H = D // n; hm = bm // n
    nb = B // bm
    rr = H // nb
    def kern(x0_hbm, w_hbm, b_ref, o_hbm, x0v, xv, wv, sv, bv, xsem, wsem, osem):
        xc = lambda i: pltpu.make_async_copy(x0_hbm.at[pl.ds(i * bm, bm)], x0v.at[pl.ds(i * bm, bm)], xsem.at[i])
        wc = lambda l: pltpu.make_async_copy(w_hbm.at[l], wv.at[l], wsem.at[l])
        oc = lambda i: pltpu.make_async_copy(xv.at[pl.ds(i * bm, bm)], o_hbm.at[pl.ds(i * bm, bm)], osem.at[i])
        wc(0).start(); xc(0).start()
        for l in range(L): bv[l] = b_ref[l:l + 1, :].astype(f32)
        wc(0).wait()
        wc(1).start()
        def wprep(l, slot, r0, rows):
            blk = [[wv[l, pl.ds(i * H + r0, rows), j * H:(j + 1) * H].astype(f32) for j in range(n)] for i in range(n)]
            for p, t in enumerate(combos(blk, BC)):
                sv[slot, p, pl.ds(r0, rows), :] = t.astype(bf16)
        @pl.loop(0, H // 32)
        def _(r): wprep(0, 0, pl.multiple_of(r * 32, 32), 32)
        def step(l, i, src):
            r0 = pl.multiple_of(i * bm, bm)
            slot = l % 2
            a = [[src[pl.ds(r0 + p * hm, hm), q * H:(q + 1) * H].astype(f32) for q in range(n)] for p in range(n)]
            it = (jnp.dot(t.astype(bf16), sv[slot, p], preferred_element_type=f32) for p, t in enumerate(combos(a, AC)))
            C = products(n, it)
            for p in range(n):
                for q in range(n):
                    rs = pl.ds(r0 + p * hm, hm); cs = slice(q * H, (q + 1) * H)
                    xv[rs, cs] = (x0v[rs, cs].astype(f32) * (C[p][q] + bv[l, :, cs]) + a[p][q]).astype(bf16)
            ln = jnp.minimum(l + 1, L - 1)
            wprep(ln, 1 - slot, pl.multiple_of(i * rr, rr), rr)
        wc(1).wait()
        for i in range(1, nb): xc(i).start()
        @pl.loop(0, nb)
        def _(i):
            xc(i).wait()
            @pl.when(i == 1)
            def _():
                for l in range(2, L): wc(l).start()
            step(0, i, x0v)
        @pl.loop(1, L)
        def _(l):
            @pl.when(l + 1 < L)
            def _(): wc(l + 1).wait()
            @pl.loop(0, nb)
            def _(i):
                step(l, i, xv)
                @pl.when(l == L - 1)
                def _(): oc(i).start()
        for i in range(nb): oc(i).wait()
    return pl.pallas_call(
        kern,
        in_specs=[pl.BlockSpec(memory_space=pltpu.HBM), pl.BlockSpec(memory_space=pltpu.HBM), pl.BlockSpec(memory_space=pltpu.VMEM)],
        out_specs=pl.BlockSpec(memory_space=pltpu.HBM),
        out_shape=jax.ShapeDtypeStruct((B, D), bf16),
        scratch_shapes=[pltpu.VMEM((B, D), bf16), pltpu.VMEM((B, D), bf16), pltpu.VMEM((L, D, D), bf16), pltpu.VMEM((2, P, H, H), bf16), pltpu.VMEM((L, 1, D), f32),
                        pltpu.SemaphoreType.DMA((nb,)), pltpu.SemaphoreType.DMA((L,)), pltpu.SemaphoreType.DMA((nb,))],
        compiler_params=pltpu.CompilerParams(vmem_limit_bytes=100 * 2**20, disable_bounds_checks=True),
    )(x0, ws, bs)
```
